```python
import os as _os
_os.environ.setdefault("JAX_PLATFORMS", "cpu")
import jax
import jax.numpy as jnp

def _softmax(x, axis=-1):
    return jax.nn.softmax(x, axis=axis)
def _gelu(x):
    return jax.nn.gelu(x, approximate=True)
def _silu(x):
    return jax.nn.silu(x)
def _sigmoid(x):
    return jax.nn.sigmoid(x)
def _layernorm(x, axis=-1, eps=1e-5):
    m = jnp.mean(x, axis=axis, keepdims=True)
    v = jnp.var(x, axis=axis, keepdims=True)
    return (x - m) / jnp.sqrt(v + eps)
def _scatter_add(tgt, idx, src, axis=0):
    return tgt.at[idx].add(src)
def _segment_sum(src, seg, n):
    return jax.ops.segment_sum(src, seg, n)
class _Rng:
    def __init__(self, key):
        self._k = key
    def _next(self):
        self._k, sub = jax.random.split(self._k)
        return sub
    def normal(self, shape):
        return jax.random.normal(self._next(), shape, dtype=jnp.bfloat16)
    def randint(self, lo, hi, shape):
        return jax.random.randint(self._next(), shape, lo, hi, dtype=jnp.int32)
    def uniform(self, shape, lo=0.0, hi=1.0):
        return jax.random.uniform(self._next(), shape, jnp.bfloat16, lo, hi)
    def permutation(self, n):
        return jax.random.permutation(self._next(), n)


kernel_name = 'parallel_sum__softmax_full_mha__moe_arch_mod__prompt'

def setup_inputs():
    _rng = _Rng(jax.random.key(int.from_bytes(__import__("os").urandom(4), "little")))
    _w = (lambda a: (lambda t: t.astype(jnp.bfloat16) if jnp.issubdtype(t.dtype, jnp.floating) else t)(jnp.asarray(a)))
    def _A_setup():
        B, S, D = 1, 2048, 512
        return {
            "x": _w((lambda *s: _rng.normal(s) * 0.05)(B, S, D)),
            "wqkv": _w((lambda *s: _rng.normal(s) * 0.1)(D, 3 * D)),
            "wo": _w((lambda *s: _rng.normal(s) * 0.05)(D, D)),
        }
    _A_in = _A_setup()

    def _B_setup():
        B, S, D, F, C = 1, 2048, 512, 1792, 1
        return {
            "x": _w((lambda *s: _rng.normal(s) * 0.05)(B, S, D)),
            "w_r": _w((lambda *s: _rng.normal(s) * 1.6)(D)),
            "w_gate": _w((lambda *s: _rng.normal(s) * 0.1)(D, F)),
            "w_up": _w((lambda *s: _rng.normal(s) * 0.1)(D, F)),
            "w_down": _w((lambda *s: _rng.normal(s) * 0.1)(F, D)),
        }
    _B_in = _B_setup()

    return {
        "A_x": _A_in["x"],
        "A_wqkv": _A_in["wqkv"],
        "A_wo": _A_in["wo"],
        "B_x": _B_in["x"],
        "B_w_r": _B_in["w_r"],
        "B_w_gate": _B_in["w_gate"],
        "B_w_up": _B_in["w_up"],
        "B_w_down": _B_in["w_down"],
    }

def reference(A_x, A_wqkv, A_wo, B_x, B_w_r, B_w_gate, B_w_up, B_w_down):
    def _A_ref(x, wqkv, wo):
        B, S, D = x.shape
        H = 32; Dh = D // H
        qkv = (lambda x, *d: x.transpose(*d))((x @ wqkv).reshape(B, S, 3, H, Dh), 2, 0, 3, 1, 4)
        q, k, v = qkv[0], qkv[1], qkv[2]
        scale = Dh ** -0.5
        scores = jnp.einsum("bhqd,bhkd->bhqk", q, k) * scale
        p = _softmax(scores, axis=-1)
        o = jnp.einsum("bhqk,bhkd->bhqd", p, v)
        return (lambda x, *d: x.transpose(*d))(o, 0, 2, 1, 3).reshape(B, S, D) @ wo

    def _B_ref(x, w_r, w_gate, w_up, w_down):
        B, S, D = x.shape
        C = 1
        r = x @ w_r
        idx = jnp.argsort(-r, axis=-1)[:, :C]
        idx_e = jnp.repeat(idx.reshape(B, C, 1), D, axis=2)
        x_sel = jnp.take_along_axis(x, idx_e, axis=1)
        g = _silu(x_sel @ w_gate)
        u = x_sel @ w_up
        y = (g * u) @ w_down
        r_sel = _sigmoid(jnp.take_along_axis(r, idx, axis=1))
        y = y * r_sel.reshape(B, C, 1)
        b_off = (jnp.arange(B) * S).reshape(B, 1)
        flat_idx = (idx + b_off).reshape(B * C)
        zero = (x * 0.0).reshape(B * S, D)
        upd = _scatter_add(zero, flat_idx, y.reshape(B * C, D), axis=0)
        return x + upd.reshape(B, S, D)

    x = A_x
    xn = _layernorm(x, axis=-1)
    return x + _A_ref(xn, A_wqkv, A_wo) + _B_ref(xn, B_w_r, B_w_gate, B_w_up, B_w_down)
```

```python
import jax
import jax.numpy as jnp
import numpy as np
import jax.experimental.pallas as pl
import jax.experimental.pallas.tpu as pltpu

S, D, H, DH, F = 2048, 512, 32, 16, 1792
BQ = 512
CK = 128
NQT = BQ // 128
NCK = S // CK
NQB = S // BQ
N_ITEMS = NQB * H
RC = 256
NRC = S // RC
LOG2E = 1.4426950408889634
QSCALE = float(DH ** -0.5 * LOG2E)
EPS_BF16 = float(np.asarray(1e-5, dtype=jnp.bfloat16).astype(np.float32))

f32 = jnp.float32
bf16 = jnp.bfloat16


def _rb(a):
    return a.astype(bf16).astype(f32)


def make(flags=None, nblocks=None):
    def kernel(x_hbm, wqkv_hbm, wo_hbm, wr_ref, wg_hbm, wu_hbm, wd_hbm, out_hbm,
               x_v, wq_v, wk_v, wv_v, wo_v, wg_v, wu_v, wd_v, wt_v,
               xn_s, k_s, qt_s, vt_s, ot_s, r_s, sa0, sa1, sb0, sb1, out_v, sems, osems):
        def xcopy(c):
            return pltpu.make_async_copy(x_hbm.at[c * RC:(c + 1) * RC, :], x_v.at[c * RC:(c + 1) * RC, :], sems.at[c])
        cp_k = pltpu.make_async_copy(wqkv_hbm.at[:, D:2 * D], wk_v, sems.at[NRC])
        cp_q = pltpu.make_async_copy(wqkv_hbm.at[:, 0:D], wq_v, sems.at[NRC + 1])
        cp_v = pltpu.make_async_copy(wqkv_hbm.at[:, 2 * D:3 * D], wv_v, sems.at[NRC + 2])
        cp_o = pltpu.make_async_copy(wo_hbm, wo_v, sems.at[NRC + 3])
        cp_g = pltpu.make_async_copy(wg_hbm, wg_v, sems.at[NRC + 4])
        cp_u = pltpu.make_async_copy(wu_hbm, wu_v, sems.at[NRC + 5])
        cp_d = pltpu.make_async_copy(wd_hbm, wd_v, sems.at[NRC + 6])
        xcopy(0).start()
        cp_k.start()
        cp_q.start()
        cp_v.start()
        for c in range(1, NRC):
            xcopy(c).start()
        cp_g.start()
        cp_u.start()
        cp_d.start()
        cp_o.start()

        def ln(c):
            xcopy(c).wait()
            x = x_v[c * RC:(c + 1) * RC, :].astype(f32)
            mean = jnp.sum(x, axis=1, keepdims=True) * (1.0 / D)
            xc = x - mean
            var = jnp.sum(xc * xc, axis=1, keepdims=True) * (1.0 / D)
            d = _rb(x - _rb(mean))
            sd = _rb(jnp.sqrt(_rb(_rb(var) + EPS_BF16)))
            xn = (d * (1.0 / sd)).astype(bf16)
            xn_s[c * RC:(c + 1) * RC, :] = xn
            return xn

        def kproj(c, xn):
            kk = jnp.dot(xn, wk_v[...], preferred_element_type=f32).astype(bf16)
            for g in range(D // 128):
                k_s[g, c * RC:(c + 1) * RC, :] = kk[:, g * 128:(g + 1) * 128]

        def qvproj(c, xn):
            t = jax.lax.dot_general(wt_v[...], xn, (((1,), (1,)), ((), ())), preferred_element_type=f32)
            qt_s[:, c * RC:(c + 1) * RC] = (t[0:D] * QSCALE).astype(bf16)
            vt_s[:, c * RC:(c + 1) * RC] = t[D:2 * D].astype(bf16)
            r_s[:, c * RC:(c + 1) * RC] = t[2 * D:2 * D + 8]

        xn = ln(0)
        cp_k.wait()
        kproj(0, xn)
        cp_q.wait()
        wt_v[0:D, :] = wq_v[...].T
        cp_v.wait()
        wt_v[D:2 * D, :] = wv_v[...].T
        wt_v[2 * D:2 * D + 16, :] = jnp.broadcast_to(wr_ref[...].reshape(1, D), (16, D))
        for c in range(NRC):
            if c + 1 < NRC:
                xn_next = ln(c + 1)
            qvproj(c, xn)
            if c + 1 < NRC:
                kproj(c + 1, xn_next)
                xn = xn_next

        rows = jax.lax.broadcasted_iota(jnp.int32, (128, BQ), 0)

        def make_rhs(item):
            h = item % H
            q0 = pl.multiple_of((item // H) * BQ, BQ)
            g = h // 8
            qt = qt_s[pl.ds(pl.multiple_of(g * 128, 128), 128), pl.ds(q0, BQ)]
            return g, jnp.where(rows // DH == h % 8, qt, jnp.zeros_like(qt))

        def qk_chunk(g, rhs, buf, c, m):
            s = jnp.dot(k_s[g, c * CK:(c + 1) * CK, :], rhs, preferred_element_type=f32)
            buf[c * CK:(c + 1) * CK, :] = s
            for t in range(NQT):
                for r in range(CK // 8):
                    sl = s[r * 8:(r + 1) * 8, t * 128:(t + 1) * 128]
                    m[t] = sl if m[t] is None else jnp.maximum(m[t], sl)

        def pv_chunk(r0, buf, c, mcur, acc, l, off):
            vt = vt_s[pl.ds(r0, DH), c * CK:(c + 1) * CK]
            for t in range(NQT):
                if off is None:
                    sv = buf[c * CK:(c + 1) * CK, t * 128:(t + 1) * 128]
                else:
                    sv = buf[pl.ds(pl.multiple_of(off + c * CK, 8), CK), t * 128:(t + 1) * 128]
                p = jnp.exp2(sv - mcur[t])
                for r in reversed(range(CK // 8)):
                    l[t] = p[r * 8:(r + 1) * 8] if l[t] is None else l[t] + p[r * 8:(r + 1) * 8]
                d = jnp.dot(vt, p.astype(bf16), preferred_element_type=f32)
                acc[t] = d if acc[t] is None else acc[t] + d

        def fin_m(m):
            return [jnp.max(x, axis=0, keepdims=True) for x in m]

        def sub(pv_item, pv_buf, mcur, qk_item, qk_buf, off):
            acc, l, m = [None] * NQT, [None] * NQT, [None] * NQT
            if qk_item is not None:
                g, rhs = make_rhs(qk_item)
            if pv_item is not None:
                r0 = pl.multiple_of((pv_item % H) * DH, DH)
            for c in range(NCK):
                if qk_item is not None:
                    qk_chunk(g, rhs, qk_buf, c, m)
                if pv_item is not None:
                    pv_chunk(r0, pv_buf, c, mcur, acc, l, off)
            if pv_item is not None:
                o = jnp.concatenate([a / jnp.sum(x, axis=0, keepdims=True) for a, x in zip(acc, l)], axis=1)
                q0 = pl.multiple_of((pv_item // H) * BQ, BQ)
                ot_s[pl.ds(r0, DH), pl.ds(q0, BQ)] = o.astype(bf16)
            if qk_item is not None:
                return fin_m(m)

        ma0 = sub(None, None, None, 0, sa0, None)
        ma1 = sub(None, None, None, 1, sa1, None)

        r = r_s[0:1, :]
        r = _rb(r)
        rmax = jnp.max(r, axis=1, keepdims=True)
        lane = jax.lax.broadcasted_iota(jnp.int32, (1, S), 1)
        idx = jnp.min(jnp.where(r == rmax, lane, S - 1))
        idx = jnp.clip(idx, 0, S - 1)
        base = pl.multiple_of((idx // 16) * 16, 16)
        xs = xn_s[pl.ds(base, 16), :]
        cp_g.wait()
        cp_u.wait()
        gg = jnp.dot(xs, wg_v[...], preferred_element_type=f32)
        uu = jnp.dot(xs, wu_v[...], preferred_element_type=f32)
        hh = (gg * (1.0 / (1.0 + jnp.exp(-gg))) * uu).astype(bf16)
        cp_d.wait()
        y = jnp.dot(hh, wd_v[...], preferred_element_type=f32)
        sel = jax.lax.broadcasted_iota(jnp.int32, (16, D), 0) == idx - base
        yrow = jnp.sum(jnp.where(sel, y, 0.0), axis=0, keepdims=True)
        yrow = yrow * (1.0 / (1.0 + jnp.exp(-rmax)))

        def body(b, carry):
            m0, m1 = carry
            i = b * 4
            off = (b >> 20) * 8
            mb0 = sub(i, sa0, m0, i + 2, sb0, None)
            mb1 = sub(i + 1, sa1, m1, i + 3, sb1, None)
            m0 = sub(i + 2, sb0, mb0, i + 4, sa0, off)
            m1 = sub(i + 3, sb1, mb1, i + 5, sa1, off)
            return m0, m1

        nb = N_ITEMS // 4 - 1 if nblocks is None else nblocks
        m0, m1 = jax.lax.fori_loop(0, nb, body, (ma0, ma1))
        i = N_ITEMS - 4
        off = (idx >> 20) * 8
        mb0 = sub(i, sa0, m0, i + 2, sb0, None)
        mb1 = sub(i + 1, sa1, m1, i + 3, sb1, None)
        sub(i + 2, sb0, mb0, None, None, off)
        sub(i + 3, sb1, mb1, None, None, off)

        cp_o.wait()
        ocs = []
        for c in range(NRC):
            sl = slice(c * RC, (c + 1) * RC)
            a = jax.lax.dot_general(ot_s[:, sl], wo_v[...], (((0,), (0,)), ((), ())), preferred_element_type=f32)
            rowid = jax.lax.broadcasted_iota(jnp.int32, (RC, D), 0) + c * RC
            o = x_v[sl, :].astype(f32) + a + (xn_s[sl, :].astype(f32) + jnp.where(rowid == idx, yrow, 0.0))
            out_v[sl, :] = o.astype(bf16)
            cp = pltpu.make_async_copy(out_v.at[sl, :], out_hbm.at[sl, :], osems.at[c])
            cp.start()
            ocs.append(cp)
        for cp in ocs:
            cp.wait()

    @jax.jit
    def fn(A_x, A_wqkv, A_wo, B_x, B_w_r, B_w_gate, B_w_up, B_w_down):
        anyspec = pl.BlockSpec(memory_space=pl.ANY)
        out = pl.pallas_call(
            kernel,
            out_shape=jax.ShapeDtypeStruct((S, D), bf16),
            in_specs=[anyspec, anyspec, anyspec, pl.BlockSpec(memory_space=pltpu.VMEM), anyspec, anyspec, anyspec],
            out_specs=anyspec,
            scratch_shapes=[
                pltpu.VMEM((S, D), bf16), pltpu.VMEM((D, D), bf16), pltpu.VMEM((D, D), bf16), pltpu.VMEM((D, D), bf16),
                pltpu.VMEM((D, D), bf16), pltpu.VMEM((D, F), bf16), pltpu.VMEM((D, F), bf16), pltpu.VMEM((F, D), bf16),
                pltpu.VMEM((2 * D + 16, D), bf16),
                pltpu.VMEM((S, D), bf16), pltpu.VMEM((D // 128, S, 128), bf16), pltpu.VMEM((D, S), bf16),
                pltpu.VMEM((D, S), bf16), pltpu.VMEM((D, S), bf16), pltpu.VMEM((8, S), f32),
                pltpu.VMEM((S, BQ), f32), pltpu.VMEM((S, BQ), f32), pltpu.VMEM((S, BQ), f32), pltpu.VMEM((S, BQ), f32),
                pltpu.VMEM((S, D), bf16),
                pltpu.SemaphoreType.DMA((NRC + 7,)), pltpu.SemaphoreType.DMA((NRC,)),
            ],
            compiler_params=pltpu.CompilerParams(vmem_limit_bytes=100 * 1024 * 1024, flags=flags),
        )(A_x.reshape(S, D), A_wqkv, A_wo, B_w_r, B_w_gate, B_w_up, B_w_down)
        return out.reshape(A_x.shape)

    return fn


pallas_parallel_sum__softmax_full_mha__moe_arch_mod__prompt_kernel = make()
```

```python
import jax
import jax.numpy as jnp
import numpy as np
import jax.experimental.pallas as pl
import jax.experimental.pallas.tpu as pltpu

S, D, H, DH, F = 2048, 512, 32, 16, 1792
BQ = 512
CK = 128
NQT = BQ // 128
NCK = S // CK
NQB = S // BQ
HPS = 8
NG = H // HPS
NB = NQB * NG
RC = 256
NRC = S // RC
VO = 16
LOG2E = 1.4426950408889634
QSCALE = float(DH ** -0.5 * LOG2E)
EPS_BF16 = float(np.asarray(1e-5, dtype=jnp.bfloat16).astype(np.float32))

f32 = jnp.float32
bf16 = jnp.bfloat16


def _rb(a):
    return a.astype(bf16).astype(f32)


def make(flags=None, nblocks=None, ffn_start=16, dphase=1, npairs=7, dsplit=8, dper=10):
    def kernel(x_hbm, wqkv_hbm, wo_hbm, wr_hbm, wg_hbm, wu_hbm, wd_hbm, out_hbm,
               x_v, wq_v, wk_v, wv_v, wo_v, wg_v, wu_v, wd_v, wt_v,
               xn_s, k_s, qt_s, vt_s, ot_s, r_s, sbuf, qb_s, kf_s, wr_v, out_v, sems, osems):
        def xcopy(c):
            return pltpu.make_async_copy(x_hbm.at[c * RC:(c + 1) * RC, :], x_v.at[c * RC:(c + 1) * RC, :], sems.at[c])
        cp_k = pltpu.make_async_copy(wqkv_hbm.at[:, D:2 * D], wk_v, sems.at[NRC])
        cp_q = pltpu.make_async_copy(wqkv_hbm.at[:, 0:D], wq_v, sems.at[NRC + 1])
        cp_v = pltpu.make_async_copy(wqkv_hbm.at[:, 2 * D:3 * D], wv_v, sems.at[NRC + 2])
        cp_o = pltpu.make_async_copy(wo_hbm, wo_v, sems.at[NRC + 3])
        cp_g = pltpu.make_async_copy(wg_hbm, wg_v, sems.at[NRC + 4])
        cp_u = pltpu.make_async_copy(wu_hbm, wu_v, sems.at[NRC + 5])
        cp_d = pltpu.make_async_copy(wd_hbm, wd_v, sems.at[NRC + 6])
        xcopy(0).start()
        cp_k.start()
        xcopy(1).start()
        cp_q.start()
        xcopy(2).start()
        cp_v.start()
        cp_r = pltpu.make_async_copy(wr_hbm, wr_v, sems.at[NRC + 7])
        cp_r.start()
        for c in range(3, NRC):
            xcopy(c).start()
        cp_g.start()
        cp_u.start()
        cp_d.start()
        cp_o.start()

        def ln(c):
            x = x_v[c * RC:(c + 1) * RC, :].astype(f32)
            mean = jnp.sum(x, axis=1, keepdims=True) * (1.0 / D)
            xc = x - mean
            var = jnp.sum(xc * xc, axis=1, keepdims=True) * (1.0 / D)
            d = _rb(x - _rb(mean))
            sd = _rb(jnp.sqrt(_rb(_rb(var) + EPS_BF16)))
            xn = (d * (1.0 / sd)).astype(bf16)
            xn_s[c * RC:(c + 1) * RC, :] = xn
            return xn

        def kproj(c, xn):
            kk = jnp.dot(xn, wk_v[...], preferred_element_type=f32).astype(bf16)
            for g in range(D // 128):
                kg = kk[:, g * 128:(g + 1) * 128]
                k_s[g, c * RC // 2:(c + 1) * RC // 2, :] = pltpu.bitcast(kg, jnp.uint32)
                kf_s[g, c * VO:(c + 1) * VO, :] = kg[RC - VO:].astype(f32)

        def qvproj(c, xn):
            t = jax.lax.dot_general(wt_v[...], xn, (((1,), (1,)), ((), ())), preferred_element_type=f32)
            qt_s[:, c * RC:(c + 1) * RC] = (t[0:D] * QSCALE).astype(bf16)
            vt_s[:, c * RC:(c + 1) * RC] = t[D:2 * D].astype(bf16)
            r_s[:, c * RC:(c + 1) * RC] = t[2 * D:2 * D + 8]

        def xs_(c):
            return xn_s[c * RC:(c + 1) * RC, :]

        xcopy(0).wait()
        ln(0)
        cp_k.wait()
        xcopy(1).wait()
        ln(1)
        kproj(0, xs_(0))
        cp_q.wait()
        xcopy(2).wait()
        ln(2)
        wt_v[0:D, :] = wq_v[...].T
        kproj(1, xs_(1))
        cp_v.wait()
        cp_r.wait()
        xcopy(3).wait()
        ln(3)
        wt_v[D:2 * D, :] = wv_v[...].T
        wt_v[2 * D:2 * D + 16, :] = jnp.broadcast_to(wr_v[...].reshape(1, D), (16, D))
        kproj(2, xs_(2))
        kproj(3, xs_(3))
        qvproj(0, xs_(0))
        for c in range(4, NRC):
            xcopy(c).wait()
        for c in range(4, NRC):
            ln(c)
            qvproj(c - 3, xs_(c - 3))
            kproj(c, xs_(c))
        for c in range(NRC - 3, NRC):
            qvproj(c, xs_(c))

        def q_tile(blk, hh):
            q0 = pl.multiple_of((blk // NG) * BQ, BQ)
            return qt_s[pl.ds(pl.multiple_of((blk % NG) * 128 + hh * DH, DH), DH), pl.ds(q0, BQ)]

        def make_rhs(blk, hh, dep):
            qt = q_tile(blk, hh)
            if dep is not None:
                lc = jnp.concatenate(dep, axis=1)
                lc = jnp.concatenate([lc, lc], axis=0)
                qt = jnp.where(lc < 0, 0.0, qt.astype(f32)).astype(bf16)
            parts = []
            if hh > 0:
                parts.append(jnp.zeros((hh * DH, BQ), bf16))
            parts.append(qt)
            if hh < HPS - 1:
                parts.append(jnp.zeros(((HPS - 1 - hh) * DH, BQ), bf16))
            return jnp.concatenate(parts, axis=0)

        def prep_qb(blk, hh, dlo, dhi):
            qf = q_tile(blk, hh).astype(f32)
            for d in range(dlo, dhi):
                qb_s[hh % 2, d] = jnp.broadcast_to(qf[d:d + 1, :], (8, BQ))

        def qk_chunk(g, rhs, hh, c, m, vacc):
            sc, ph = divmod(c, 2)
            offl = sc < npairs
            last = offl and ph == 1
            nm = CK - VO if last else CK
            kc = pltpu.bitcast(k_s[g, c * CK // 2:(c * CK + nm) // 2, :], bf16)
            s = jnp.dot(kc, rhs, preferred_element_type=f32)
            sbuf[hh, c * CK:c * CK + nm, :] = s
            for t in range(NQT):
                mc = None
                for r in range(nm // 8):
                    sl = s[r * 8:(r + 1) * 8, t * 128:(t + 1) * 128]
                    mc = sl if mc is None else jnp.maximum(mc, sl)
                m[t] = mc if m[t] is None else jnp.maximum(m[t], mc)
            if offl:
                if ph == 0:
                    vacc[0] = vacc[1] = None
                kf = kf_s[g, sc * VO:(sc + 1) * VO, :]
                for d in (range(0, dsplit) if ph == 0 else range(dsplit, DH)):
                    j = hh * DH + d
                    qb = qb_s[hh % 2, d]
                    for u in range(2):
                        pr = kf[u * 8:(u + 1) * 8, j:j + 1] * qb
                        vacc[u] = pr if vacc[u] is None else vacc[u] + pr
                if last:
                    for u in range(2):
                        sbuf[hh, c * CK + nm + u * 8:c * CK + nm + u * 8 + 8, :] = vacc[u]
                        for t in range(NQT):
                            m[t] = jnp.maximum(m[t], vacc[u][:, t * 128:(t + 1) * 128])

        def pv_chunk(r0, hh, c, mcur, acc, l):
            vt = vt_s[pl.ds(r0, DH), c * CK:(c + 1) * CK]
            for t in range(NQT):
                sv = sbuf[hh, c * CK:(c + 1) * CK, t * 128:(t + 1) * 128]
                p = jnp.exp2(sv - mcur[t])
                lc = None
                for r in reversed(range(CK // 8)):
                    lc = p[r * 8:(r + 1) * 8] if lc is None else lc + p[r * 8:(r + 1) * 8]
                l[t] = lc if l[t] is None else lc + l[t]
                d = jnp.dot(vt, p.astype(bf16), preferred_element_type=f32)
                acc[t] = d if acc[t] is None else acc[t] + d

        def block(pv_blk, mcur, qk_blk, extra=None):
            mnew = []
            for hh in range(HPS):
                acc, l, m, vacc = [None] * NQT, [None] * NQT, [None] * NQT, [None, None]
                if pv_blk is not None:
                    r0 = pl.multiple_of((pv_blk % NG) * 128 + hh * DH, DH)
                for c in range(NCK):
                    if pv_blk is not None:
                        pv_chunk(r0, hh, c, mcur[hh], acc, l)
                    if qk_blk is not None:
                        if c == 0:
                            rhs = make_rhs(qk_blk, hh, l if pv_blk is not None else None)
                        qk_chunk(qk_blk % NG, rhs, hh, c, m, vacc)
                        if c >= NCK - 2:
                            k = c - (NCK - 2)
                            if hh + 1 < HPS:
                                prep_qb(qk_blk, hh + 1, k * 8, k * 8 + 8)
                            else:
                                prep_qb(jnp.minimum(qk_blk + 1, NB - 1), 0, k * 8, k * 8 + 8)
                    if extra is not None:
                        extra(hh * NCK + c)
                if pv_blk is not None:
                    o = jnp.concatenate([a / jnp.sum(x, axis=0, keepdims=True) for a, x in zip(acc, l)], axis=1)
                    q0 = pl.multiple_of((pv_blk // NG) * BQ, BQ)
                    ot_s[pl.ds(r0, DH), pl.ds(q0, BQ)] = o.astype(bf16)
                if qk_blk is not None:
                    mnew.append([jnp.max(x, axis=0, keepdims=True) for x in m])
            return mnew

        r = r_s[0:1, :]
        r = _rb(r)
        rmax = jnp.max(r, axis=1, keepdims=True)
        lane = jax.lax.broadcasted_iota(jnp.int32, (1, S), 1)
        idx = jnp.min(jnp.where(r == rmax, lane, S - 1))
        idx = jnp.clip(idx, 0, S - 1)
        base = pl.multiple_of((idx // 16) * 16, 16)
        xs = xn_s[pl.ds(base, 16), :]
        st = {"y": None}
        NF = F // 128

        def ffn_piece(i):
            i = i - ffn_start
            if i < 0 or i >= 3 * NF + 3:
                return
            n, ph = divmod(i, 3)
            if i == 0:
                cp_g.wait()
                cp_u.wait()
                cp_d.wait()
            if ph == 0 and n < NF:
                st["g"] = jnp.dot(xs, wg_v[:, n * 128:(n + 1) * 128], preferred_element_type=f32)
            elif ph == 1 and n < NF:
                gg = st["g"]
                uu = jnp.dot(xs, wu_v[:, n * 128:(n + 1) * 128], preferred_element_type=f32)
                st["h", n] = (gg * (1.0 / (1.0 + jnp.exp(-gg))) * uu).astype(bf16)
            elif ph == 2 and n >= 1:
                d = jnp.dot(st.pop(("h", n - 1)), wd_v[(n - 1) * 128:n * 128, :], preferred_element_type=f32)
                st["y"] = d if st["y"] is None else st["y"] + d

        prep_qb(0, 0, 0, DH)
        m0 = block(None, None, 0, ffn_piece)
        sel = jax.lax.broadcasted_iota(jnp.int32, (16, D), 0) == idx - base
        yrow = jnp.sum(jnp.where(sel, st["y"], 0.0), axis=0, keepdims=True)
        yrow = yrow * (1.0 / (1.0 + jnp.exp(-rmax)))

        nb = NB - 1 if nblocks is None else nblocks
        m0 = jax.lax.fori_loop(0, nb, lambda b, m: block(b, m, b + 1), m0)

        cp_o.wait()
        ocs = []

        def finish_out(a, rows, cols, r0):
            rowid = jax.lax.broadcasted_iota(jnp.int32, a.shape, 0) + r0
            o = x_v[rows, cols].astype(f32) + a + (xn_s[rows, cols].astype(f32) + jnp.where(rowid == idx, yrow[:, cols], 0.0))
            out_v[rows, cols] = o.astype(bf16)

        def send(p):
            sl = slice(p * 128, (p + 1) * 128)
            cp = pltpu.make_async_copy(out_v.at[sl, :], out_hbm.at[sl, :], osems.at[p])
            cp.start()
            ocs.append(cp)

        n_early = (S - BQ) // 128
        ost = {}

        def drain_extra(i):
            p, ph = divmod(i, dper)
            sp = dper // 4
            if p >= n_early or ph % sp != dphase or ph // sp > 3:
                return
            n = ph // sp
            rows = slice(p * 128, (p + 1) * 128)
            cols = slice(n * 128, (n + 1) * 128)
            if n == 0:
                ost["o"] = ot_s[:, rows].T
            a = jnp.dot(ost["o"], wo_v[:, cols], preferred_element_type=f32)
            finish_out(a, rows, cols, p * 128)
            if n == 3:
                send(p)

        block(NB - 1, m0, None, drain_extra)
        for p in range(n_early, S // 128):
            rows = slice(p * 128, (p + 1) * 128)
            a = jax.lax.dot_general(ot_s[:, rows], wo_v[...], (((0,), (0,)), ((), ())), preferred_element_type=f32)
            finish_out(a, rows, slice(0, D), p * 128)
            send(p)
        for cp in ocs:
            cp.wait()

    @jax.jit
    def fn(A_x, A_wqkv, A_wo, B_x, B_w_r, B_w_gate, B_w_up, B_w_down):
        anyspec = pl.BlockSpec(memory_space=pl.ANY)
        out = pl.pallas_call(
            kernel,
            out_shape=jax.ShapeDtypeStruct((S, D), bf16),
            in_specs=[anyspec, anyspec, anyspec, anyspec, anyspec, anyspec, anyspec],
            out_specs=anyspec,
            scratch_shapes=[
                pltpu.VMEM((S, D), bf16), pltpu.VMEM((D, D), bf16), pltpu.VMEM((D, D), bf16), pltpu.VMEM((D, D), bf16),
                pltpu.VMEM((D, D), bf16), pltpu.VMEM((D, F), bf16), pltpu.VMEM((D, F), bf16), pltpu.VMEM((F, D), bf16),
                pltpu.VMEM((2 * D + 16, D), bf16),
                pltpu.VMEM((S, D), bf16), pltpu.VMEM((D // 128, S // 2, 128), jnp.uint32), pltpu.VMEM((D, S), bf16),
                pltpu.VMEM((D, S), bf16), pltpu.VMEM((D, S), bf16), pltpu.VMEM((8, S), f32),
                pltpu.VMEM((HPS, S, BQ), f32), pltpu.VMEM((2, DH, 8, BQ), f32), pltpu.VMEM((NG, NRC * VO, 128), f32), pltpu.VMEM((D,), bf16),
                pltpu.VMEM((S, D), bf16),
                pltpu.SemaphoreType.DMA((NRC + 8,)), pltpu.SemaphoreType.DMA((S // 128,)),
            ],
            compiler_params=pltpu.CompilerParams(vmem_limit_bytes=100 * 1024 * 1024, flags=flags),
        )(A_x.reshape(S, D), A_wqkv, A_wo, B_w_r, B_w_gate, B_w_up, B_w_down)
        return out.reshape(A_x.shape)

    return fn


pallas_parallel_sum__softmax_full_mha__moe_arch_mod__prompt_kernel = make()
```
